```python
import os as _os
_os.environ.setdefault("JAX_PLATFORMS", "cpu")
import jax
import jax.numpy as jnp

def _softmax(x, axis=-1):
    return jax.nn.softmax(x, axis=axis)
def _gelu(x):
    return jax.nn.gelu(x, approximate=True)
def _silu(x):
    return jax.nn.silu(x)
def _sigmoid(x):
    return jax.nn.sigmoid(x)
def _layernorm(x, axis=-1, eps=1e-5):
    m = jnp.mean(x, axis=axis, keepdims=True)
    v = jnp.var(x, axis=axis, keepdims=True)
    return (x - m) / jnp.sqrt(v + eps)
def _scatter_add(tgt, idx, src, axis=0):
    return tgt.at[idx].add(src)
def _segment_sum(src, seg, n):
    return jax.ops.segment_sum(src, seg, n)
class _Rng:
    def __init__(self, key):
        self._k = key
    def _next(self):
        self._k, sub = jax.random.split(self._k)
        return sub
    def normal(self, shape):
        return jax.random.normal(self._next(), shape, dtype=jnp.bfloat16)
    def randint(self, lo, hi, shape):
        return jax.random.randint(self._next(), shape, lo, hi, dtype=jnp.int32)
    def uniform(self, shape, lo=0.0, hi=1.0):
        return jax.random.uniform(self._next(), shape, jnp.bfloat16, lo, hi)
    def permutation(self, n):
        return jax.random.permutation(self._next(), n)


kernel_name = 'concat_heads__sliding_block_cached__sliding_block_cached__decode'

def setup_inputs():
    _rng = _Rng(jax.random.key(int.from_bytes(__import__("os").urandom(4), "little")))
    _w = (lambda a: (lambda t: t.astype(jnp.bfloat16) if jnp.issubdtype(t.dtype, jnp.floating) else t)(jnp.asarray(a)))
    def _A_setup():
        B, Sq, D = 2, 1, 640
        Hq, Hkv, Sk, Dh = 32, 32, 4096, 128
        assert Hq % Hkv == 0, (Hq, Hkv)
        return {
            "x": _w((lambda *s: _rng.normal(s) * 0.8)(B, Sq, D)),
            "k_cache": _w((lambda *s: _rng.normal(s) * 0.8)(B, Hkv, Sk, Dh)),
            "v_cache": _w((lambda *s: _rng.normal(s) * 0.05)(B, Hkv, Sk, Dh)),
            "wq": _w((lambda *s: _rng.normal(s) * 0.8)(D, Hq * Dh) * (D ** -0.5)),
            "wo": _w((lambda *s: _rng.normal(s) * 0.05)(Hq * Dh, D) * ((Hq * Dh) ** -0.5)),
        }
    _A_in = _A_setup()

    def _B_setup():
        B, Sq, D = 2, 1, 640
        Hq, Hkv, Sk, Dh = 32, 32, 4096, 128
        assert Hq % Hkv == 0, (Hq, Hkv)
        return {
            "x": _w((lambda *s: _rng.normal(s) * 0.8)(B, Sq, D)),
            "k_cache": _w((lambda *s: _rng.normal(s) * 0.8)(B, Hkv, Sk, Dh)),
            "v_cache": _w((lambda *s: _rng.normal(s) * 0.05)(B, Hkv, Sk, Dh)),
            "wq": _w((lambda *s: _rng.normal(s) * 0.8)(D, Hq * Dh) * (D ** -0.5)),
            "wo": _w((lambda *s: _rng.normal(s) * 0.05)(Hq * Dh, D) * ((Hq * Dh) ** -0.5)),
        }
    _B_in = _B_setup()

    return {
        "A_x": _A_in["x"],
        "A_k_cache": _A_in["k_cache"],
        "A_v_cache": _A_in["v_cache"],
        "A_wq": _A_in["wq"],
        "A_wo": _A_in["wo"],
        "B_x": _B_in["x"],
        "B_k_cache": _B_in["k_cache"],
        "B_v_cache": _B_in["v_cache"],
        "B_wq": _B_in["wq"],
        "B_wo": _B_in["wo"],
    }

def reference(A_x, A_k_cache, A_v_cache, A_wq, A_wo, B_x, B_k_cache, B_v_cache, B_wq, B_wo):
    def _A_ref(x, k_cache, v_cache, wq, wo):
        B, Sq, D = x.shape
        Hq, Dh = 32, 128
        Hkv, Sk = k_cache.shape[1], k_cache.shape[2]
        W = min(4096, max(256, Sk // 4))
        rep = Hq // Hkv
        q = (lambda x, *d: x.transpose(*d))((x @ wq).reshape(B, Sq, Hq, Dh), 0, 2, 1, 3)
        k = jnp.repeat(k_cache[:, :, Sk - W:, :], rep, axis=1)
        v = jnp.repeat(v_cache[:, :, Sk - W:, :], rep, axis=1)
        scores = jnp.einsum("bhqd,bhkd->bhqk", q, k) * (Dh ** -0.5)
        p = _softmax(scores, axis=-1)
        o = jnp.einsum("bhqk,bhkd->bhqd", p, v)
        return (lambda x, *d: x.transpose(*d))(o, 0, 2, 1, 3).reshape(B, Sq, Hq * Dh) @ wo

    def _B_ref(x, k_cache, v_cache, wq, wo):
        B, Sq, D = x.shape
        Hq, Dh = 32, 128
        Hkv, Sk = k_cache.shape[1], k_cache.shape[2]
        W = min(4096, max(256, Sk // 4))
        rep = Hq // Hkv
        q = (lambda x, *d: x.transpose(*d))((x @ wq).reshape(B, Sq, Hq, Dh), 0, 2, 1, 3)
        k = jnp.repeat(k_cache[:, :, Sk - W:, :], rep, axis=1)
        v = jnp.repeat(v_cache[:, :, Sk - W:, :], rep, axis=1)
        scores = jnp.einsum("bhqd,bhkd->bhqk", q, k) * (Dh ** -0.5)
        p = _softmax(scores, axis=-1)
        o = jnp.einsum("bhqk,bhkd->bhqd", p, v)
        return (lambda x, *d: x.transpose(*d))(o, 0, 2, 1, 3).reshape(B, Sq, Hq * Dh) @ wo

    a = _A_ref(A_x, A_k_cache, A_v_cache, A_wq, A_wo)
    b = _B_ref(B_x, B_k_cache, B_v_cache, B_wq, B_wo)
    return jnp.concatenate([a, b], axis=-1)
```

```python
import jax
import jax.numpy as jnp
from jax import lax
import jax.experimental.pallas as pl
import jax.experimental.pallas.tpu as pltpu

_B, _D = 2, 640
_H, _SK, _DH = 32, 4096, 128
_W = min(4096, max(256, _SK // 4))
_G = 4
_R = 2 * _G
_NT = (((1,), (1,)), ((), ()))

_SCHEDULE = (
    ("wq", 0, 0, 0), ("x", 0, 0, 0), ("x", 1, 0, 0), ("wq", 1, 0, 0),
    ("k", 0, 0, _H), ("v", 0, 0, _H),
    ("k", 1, 0, _H), ("v", 1, 0, _H),
    ("wo", 0, 0, _H),
    ("wo", 1, 0, 24), ("wo", 1, 24, 7), ("wo", 1, 31, 1),
)


def _kernel(ax, ak, av, awq, awo, bx, bk, bv, bwq, bwo, o_ref,
            xb, kb, vb, wqb, wob, qs, os_, sems):
    srcs = ((ax, ak, av, awq, awo), (bx, bk, bv, bwq, bwo))

    def make_copy(i):
        kind, br, h0, nh = _SCHEDULE[i]
        x_, k_, v_, wq_, wo_ = srcs[br]
        heads = pl.ds(h0, nh)
        window = pl.ds(_SK - _W, _W)
        if kind == "x":
            src, dst = x_, xb.at[br]
        elif kind == "wq":
            src, dst = wq_, wqb.at[br]
        elif kind == "k":
            src, dst = k_.at[:, heads, window, :], kb.at[br, :, heads]
        elif kind == "v":
            src, dst = v_.at[:, heads, window, :], vb.at[br, :, heads]
        else:
            rows = pl.ds(h0 * _DH, nh * _DH)
            src, dst = wo_.at[rows, :], wob.at[br, rows, :]
        return pltpu.make_async_copy(src, dst, sems.at[i])

    copies = [make_copy(i) for i in range(len(_SCHEDULE))]
    for c in copies:
        c.start()

    row = lax.broadcasted_iota(jnp.int32, (_R, 1), 0)

    def q_proj(br):
        x = xb[br].astype(jnp.float32)
        xr = jnp.where(row % 2 == 0, x[0:1], x[1:2]).astype(jnp.bfloat16)
        q = jnp.dot(xr, wqb[br], preferred_element_type=jnp.float32)
        q = q.astype(jnp.bfloat16).astype(jnp.float32)
        for h in range(_H):
            qs[br, h] = q[:, h * _DH:(h + 1) * _DH]

    def attend(br, g):
        s = None
        for j in range(_G):
            h = g * _G + j
            qj = qs[br, h].astype(jnp.bfloat16)
            for b in range(_B):
                sj = lax.dot_general(qj, kb[br, b, h], _NT,
                                     preferred_element_type=jnp.float32)
                s = sj if s is None else jnp.where(row == 2 * j + b, sj, s)
        s = s * (_DH ** -0.5)
        p = jnp.exp(s - jnp.max(s, axis=-1, keepdims=True))
        l = jnp.sum(p, axis=-1, keepdims=True)
        pb = p.astype(jnp.bfloat16)
        o = None
        for j in range(_G):
            h = g * _G + j
            for b in range(_B):
                oj = jnp.dot(pb, vb[br, b, h], preferred_element_type=jnp.float32)
                o = oj if o is None else jnp.where(row == 2 * j + b, oj, o)
        o = o / l
        for j in range(_G):
            os_[br, g * _G + j] = o if j == 0 else pltpu.roll(o, _R - 2 * j, 0)

    def o_proj(br, h0, nh, acc):
        def one(h, a):
            r0 = h * _DH if isinstance(h, int) else pl.multiple_of(h * _DH, _DH)
            return a + jnp.dot(os_[br, h].astype(jnp.bfloat16),
                               wob[br, pl.ds(r0, _DH), :],
                               preferred_element_type=jnp.float32)

        u = 8
        n_loop = nh // u
        done = 0
        if n_loop > 1:
            def body(i, a):
                for jj in range(u):
                    a = one(h0 + i * u + jj, a)
                return a
            acc = lax.fori_loop(0, n_loop, body, acc)
            done = n_loop * u
        for h in range(h0 + done, h0 + nh):
            acc = one(h, acc)
        return acc

    accs = [jnp.zeros((_R, _D), jnp.float32) for _ in range(2)]
    for i, (kind, br, h0, nh) in enumerate(_SCHEDULE):
        copies[i].wait()
        if kind == "x" and br == 0:
            q_proj(0)
        elif kind == "wq" and br == 1:
            q_proj(1)
        elif kind == "v":
            def step(g, carry, br=br):
                attend(br, g)
                return carry
            lax.fori_loop(h0 // _G, (h0 + nh) // _G, step, 0)
        elif kind == "wo":
            accs[br] = o_proj(br, h0, nh, accs[br])
    o_ref[...] = jnp.concatenate([accs[0][0:2], accs[1][0:2]], axis=-1).astype(o_ref.dtype)


@jax.jit
def pallas_concat_heads__sliding_block_cached__sliding_block_cached__decode_kernel(
    A_x: jax.Array,
    A_k_cache: jax.Array,
    A_v_cache: jax.Array,
    A_wq: jax.Array,
    A_wo: jax.Array,
    B_x: jax.Array,
    B_k_cache: jax.Array,
    B_v_cache: jax.Array,
    B_wq: jax.Array,
    B_wo: jax.Array,
):
    hbm = pl.BlockSpec(memory_space=pl.ANY)
    out = pl.pallas_call(
        _kernel,
        out_shape=jax.ShapeDtypeStruct((_B, 2 * _D), jnp.bfloat16),
        in_specs=[hbm] * 10,
        out_specs=pl.BlockSpec(memory_space=pltpu.VMEM),
        scratch_shapes=[
            pltpu.VMEM((2, _B, _D), jnp.bfloat16),
            pltpu.VMEM((2, _B, _H, _W, _DH), jnp.bfloat16),
            pltpu.VMEM((2, _B, _H, _W, _DH), jnp.bfloat16),
            pltpu.VMEM((2, _D, _H * _DH), jnp.bfloat16),
            pltpu.VMEM((2, _H * _DH, _D), jnp.bfloat16),
            pltpu.VMEM((2, _H, _R, _DH), jnp.float32),
            pltpu.VMEM((2, _H, _R, _DH), jnp.float32),
            pltpu.SemaphoreType.DMA((len(_SCHEDULE),)),
        ],
        compiler_params=pltpu.CompilerParams(vmem_limit_bytes=120 * 1024 * 1024),
    )(A_x.reshape(_B, _D), A_k_cache, A_v_cache, A_wq, A_wo,
      B_x.reshape(_B, _D), B_k_cache, B_v_cache, B_wq, B_wo)
    return out.reshape(_B, 1, 2 * _D)
```

```python
import jax
import jax.numpy as jnp
from jax import lax
import jax.experimental.pallas as pl
import jax.experimental.pallas.tpu as pltpu

_B, _D = 2, 640
_H, _SK, _DH = 32, 4096, 128
_W = min(4096, max(256, _SK // 4))
_G = 4
_R = _B * _G
_NT = (((1,), (1,)), ((), ()))

_GROUPS = (
    (("wq", 0, 0, 0), ("x", 0, 0, 0), ("x", 1, 0, 0), ("wq", 1, 0, 0)),
    (("k", 0, 0, 32), ("v", 0, 0, 32)),
    (("k", 1, 0, 16), ("v", 1, 0, 16)),
    (("k", 1, 16, 16), ("v", 1, 16, 16)),
    (("wo", 0, 0, 32),),
    (("wo", 1, 0, 20),),
    (("wo", 1, 20, 8),),
    (("wo", 1, 28, 3),),
    (("wo", 1, 31, 1),),
)
_NSEM = 3


def _kernel(ax, ak, av, awq, awo, bx, bk, bv, bwq, bwo, o_ref,
            xb, kb, vb, wqb, wob, qs, os_, sems):
    srcs = ((ax, ak, av, awq, awo), (bx, bk, bv, bwq, bwo))

    def make_copy(spec, sem):
        kind, br, h0, nh = spec
        x_, k_, v_, wq_, wo_ = srcs[br]
        heads = pl.ds(h0, nh)
        window = pl.ds(_SK - _W, _W)
        if kind == "x":
            src, dst = x_, xb.at[br]
        elif kind == "wq":
            src, dst = wq_, wqb.at[br]
        elif kind == "k":
            src, dst = k_.at[:, heads, window, :], kb.at[br, :, heads]
        elif kind == "v":
            src, dst = v_.at[:, heads, window, :], vb.at[br, :, heads]
        else:
            rows = pl.ds(h0 * _DH, nh * _DH)
            src, dst = wo_.at[rows, :], wob.at[br, rows, :]
        return pltpu.make_async_copy(src, dst, sem)

    copies = [[make_copy(spec, sems.at[i % _NSEM]) for spec in group]
              for i, group in enumerate(_GROUPS)]
    for group in copies[:_NSEM]:
        for c in group:
            c.start()

    row = lax.broadcasted_iota(jnp.int32, (_R, 1), 0)

    def q_proj(br):
        x = xb[br].astype(jnp.float32)
        xr = jnp.where(row % 2 == 0, x[0:1], x[1:2]).astype(jnp.bfloat16)
        q = jnp.dot(xr, wqb[br], preferred_element_type=jnp.float32)
        q = q.astype(jnp.bfloat16).astype(jnp.float32)
        for h in range(_H):
            qs[br, h] = q[:, h * _DH:(h + 1) * _DH]

    def attend(br, g):
        s = None
        for j in range(_G):
            h = g * _G + j
            qj = qs[br, h].astype(jnp.bfloat16)
            for b in range(_B):
                sj = lax.dot_general(qj, kb[br, b, h], _NT,
                                     preferred_element_type=jnp.float32)
                s = sj if s is None else jnp.where(row == 2 * j + b, sj, s)
        s = s * (_DH ** -0.5)
        p = jnp.exp(s - jnp.max(s, axis=-1, keepdims=True))
        l = jnp.sum(p, axis=-1, keepdims=True)
        pb = p.astype(jnp.bfloat16)
        o = None
        for j in range(_G):
            h = g * _G + j
            for b in range(_B):
                oj = jnp.dot(pb, vb[br, b, h], preferred_element_type=jnp.float32)
                o = oj if o is None else jnp.where(row == 2 * j + b, oj, o)
        o = o / l
        for j in range(_G):
            os_[br, g * _G + j] = o if j == 0 else pltpu.roll(o, _R - 2 * j, 0)

    def o_proj(br, h0, nh, acc):
        def one(h, a):
            r0 = h * _DH if isinstance(h, int) else pl.multiple_of(h * _DH, _DH)
            return a + jnp.dot(os_[br, h].astype(jnp.bfloat16),
                               wob[br, pl.ds(r0, _DH), :],
                               preferred_element_type=jnp.float32)

        u = 8
        n_loop = nh // u
        done = 0
        if n_loop > 1:
            def body(i, a):
                for jj in range(u):
                    a = one(h0 + i * u + jj, a)
                return a
            acc = lax.fori_loop(0, n_loop, body, acc)
            done = n_loop * u
        for h in range(h0 + done, h0 + nh):
            acc = one(h, acc)
        return acc

    accs = [jnp.zeros((_R, _D), jnp.float32) for _ in range(2)]
    for i, group in enumerate(_GROUPS):
        for c in copies[i]:
            c.wait()
        if i + _NSEM < len(_GROUPS):
            for c in copies[i + _NSEM]:
                c.start()
        for kind, br, h0, nh in group:
            if kind == "wq":
                q_proj(br)
            elif kind == "v":
                def step(g, carry, br=br):
                    attend(br, g)
                    return carry
                lax.fori_loop(h0 // _G, (h0 + nh) // _G, step, 0)
            elif kind == "wo":
                accs[br] = o_proj(br, h0, nh, accs[br])
    o_ref[...] = jnp.concatenate([accs[0][0:2], accs[1][0:2]], axis=-1).astype(o_ref.dtype)


@jax.jit
def pallas_concat_heads__sliding_block_cached__sliding_block_cached__decode_kernel(
    A_x: jax.Array,
    A_k_cache: jax.Array,
    A_v_cache: jax.Array,
    A_wq: jax.Array,
    A_wo: jax.Array,
    B_x: jax.Array,
    B_k_cache: jax.Array,
    B_v_cache: jax.Array,
    B_wq: jax.Array,
    B_wo: jax.Array,
):
    hbm = pl.BlockSpec(memory_space=pl.ANY)
    out = pl.pallas_call(
        _kernel,
        out_shape=jax.ShapeDtypeStruct((_B, 2 * _D), jnp.bfloat16),
        in_specs=[hbm] * 10,
        out_specs=pl.BlockSpec(memory_space=pltpu.VMEM),
        scratch_shapes=[
            pltpu.VMEM((2, _B, _D), jnp.bfloat16),
            pltpu.VMEM((2, _B, _H, _W, _DH), jnp.bfloat16),
            pltpu.VMEM((2, _B, _H, _W, _DH), jnp.bfloat16),
            pltpu.VMEM((2, _D, _H * _DH), jnp.bfloat16),
            pltpu.VMEM((2, _H * _DH, _D), jnp.bfloat16),
            pltpu.VMEM((2, _H, _R, _DH), jnp.float32),
            pltpu.VMEM((2, _H, _R, _DH), jnp.float32),
            pltpu.SemaphoreType.DMA((_NSEM,)),
        ],
        compiler_params=pltpu.CompilerParams(vmem_limit_bytes=100 * 1024 * 1024),
    )(A_x.reshape(_B, _D), A_k_cache, A_v_cache, A_wq, A_wo,
      B_x.reshape(_B, _D), B_k_cache, B_v_cache, B_wq, B_wo)
    return out.reshape(_B, 1, 2 * _D)
```

```python
import jax
import jax.numpy as jnp
from jax import lax
import jax.experimental.pallas as pl
import jax.experimental.pallas.tpu as pltpu

_B, _D = 2, 640
_H, _SK, _DH = 32, 4096, 128
_W = min(4096, max(256, _SK // 4))
_G = 4
_R = _B * _G
_NT = (((1,), (1,)), ((), ()))

_GROUPS = (
    (("wq", 0, 0, 0), ("x", 0, 0, 0), ("x", 1, 0, 0), ("wq", 1, 0, 0)),
    (("k", 0, 0, 32), ("v", 0, 0, 32)),
    (("k", 1, 0, 16), ("v", 1, 0, 16)),
    (("k", 1, 16, 16), ("v", 1, 16, 16)),
    (("wo", 0, 0, 32),),
    (("wo", 1, 0, 20),),
    (("wo", 1, 20, 8),),
    (("wo", 1, 28, 3),),
    (("wo", 1, 31, 1),),
)
_NSEM = 3


def _kernel(ax, ak, av, awq, awo, bx, bk, bv, bwq, bwo, o_ref,
            xb, kb, vb, wqb, wob, qs, os_, sems):
    srcs = ((ax, ak, av, awq, awo), (bx, bk, bv, bwq, bwo))

    def make_copy(spec, sem):
        kind, br, h0, nh = spec
        x_, k_, v_, wq_, wo_ = srcs[br]
        if kind == "x":
            src, dst = x_, xb.at[br]
        elif kind == "wq":
            src, dst = wq_, wqb.at[br]
        elif kind == "wo":
            rows = pl.ds(h0 * _DH, nh * _DH)
            src, dst = wo_.at[rows, :], wob.at[br, rows, :]
        else:
            cache, buf = (k_, kb) if kind == "k" else (v_, vb)
            heads = pl.ds(h0, nh)
            src = cache.at[:, heads, pl.ds(_SK - _W, _W), :]
            dst = buf.at[br, :, heads]
        return pltpu.make_async_copy(src, dst, sem)

    copies = [[make_copy(spec, sems.at[i % _NSEM]) for spec in group]
              for i, group in enumerate(_GROUPS)]
    for group in copies[:_NSEM]:
        for c in group:
            c.start()

    row = lax.broadcasted_iota(jnp.int32, (_R, 1), 0)

    def q_proj(br):
        x = xb[br].astype(jnp.float32)
        xr = jnp.where(row % 2 == 0, x[0:1], x[1:2]).astype(jnp.bfloat16)
        q = jnp.dot(xr, wqb[br], preferred_element_type=jnp.float32)
        q = q.astype(jnp.bfloat16).astype(jnp.float32)
        for h in range(_H):
            qs[br, h] = q[:, h * _DH:(h + 1) * _DH]

    def attend(br, g):
        s = None
        for j in range(_G):
            h = g * _G + j
            qj = qs[br, h].astype(jnp.bfloat16)
            for b in range(_B):
                sj = lax.dot_general(qj, kb[br, b, h], _NT,
                                     preferred_element_type=jnp.float32)
                s = sj if s is None else jnp.where(row == 2 * j + b, sj, s)
        s = s * (_DH ** -0.5)
        p = jnp.exp(s - jnp.max(s, axis=-1, keepdims=True))
        l = jnp.sum(p, axis=-1, keepdims=True)
        pb = p.astype(jnp.bfloat16)
        o = None
        for j in range(_G):
            h = g * _G + j
            for b in range(_B):
                oj = jnp.dot(pb, vb[br, b, h], preferred_element_type=jnp.float32)
                o = oj if o is None else jnp.where(row == 2 * j + b, oj, o)
        o = o / l
        for j in range(_G):
            os_[br, g * _G + j] = o if j == 0 else pltpu.roll(o, _R - 2 * j, 0)

    def o_proj(br, h0, nh, acc):
        def one(h, a):
            r0 = h * _DH if isinstance(h, int) else pl.multiple_of(h * _DH, _DH)
            return a + jnp.dot(os_[br, h].astype(jnp.bfloat16),
                               wob[br, pl.ds(r0, _DH), :],
                               preferred_element_type=jnp.float32)

        u = 8
        n_loop = nh // u
        done = 0
        if n_loop > 1:
            def body(i, a):
                for jj in range(u):
                    a = one(h0 + i * u + jj, a)
                return a
            acc = lax.fori_loop(0, n_loop, body, acc)
            done = n_loop * u
        for h in range(h0 + done, h0 + nh):
            acc = one(h, acc)
        return acc

    accs = [jnp.zeros((_R, _D), jnp.float32) for _ in range(2)]
    for i, group in enumerate(_GROUPS):
        for c in copies[i]:
            c.wait()
        if i + _NSEM < len(_GROUPS):
            for c in copies[i + _NSEM]:
                c.start()
        for kind, br, h0, nh in group:
            if kind == "wq":
                q_proj(br)
            elif kind == "v":
                def step(g, carry, br=br):
                    attend(br, g)
                    return carry
                lax.fori_loop(h0 // _G, (h0 + nh) // _G, step, 0)
            elif kind == "wo":
                accs[br] = o_proj(br, h0, nh, accs[br])
    o_ref[...] = jnp.concatenate([accs[0][0:2], accs[1][0:2]], axis=-1).astype(o_ref.dtype)


@jax.jit
def pallas_concat_heads__sliding_block_cached__sliding_block_cached__decode_kernel(
    A_x: jax.Array,
    A_k_cache: jax.Array,
    A_v_cache: jax.Array,
    A_wq: jax.Array,
    A_wo: jax.Array,
    B_x: jax.Array,
    B_k_cache: jax.Array,
    B_v_cache: jax.Array,
    B_wq: jax.Array,
    B_wo: jax.Array,
):
    hbm = pl.BlockSpec(memory_space=pl.ANY)
    out = pl.pallas_call(
        _kernel,
        out_shape=jax.ShapeDtypeStruct((_B, 2 * _D), jnp.bfloat16),
        in_specs=[hbm] * 10,
        out_specs=pl.BlockSpec(memory_space=pltpu.VMEM),
        scratch_shapes=[
            pltpu.VMEM((2, _B, _D), jnp.bfloat16),
            pltpu.VMEM((2, _B, _H, _W, _DH), jnp.bfloat16),
            pltpu.VMEM((2, _B, _H, _W, _DH), jnp.bfloat16),
            pltpu.VMEM((2, _D, _H * _DH), jnp.bfloat16),
            pltpu.VMEM((2, _H * _DH, _D), jnp.bfloat16),
            pltpu.VMEM((2, _H, _R, _DH), jnp.float32),
            pltpu.VMEM((2, _H, _R, _DH), jnp.float32),
            pltpu.SemaphoreType.DMA((_NSEM,)),
        ],
        compiler_params=pltpu.CompilerParams(vmem_limit_bytes=100 * 1024 * 1024),
    )(A_x.reshape(_B, _D), A_k_cache, A_v_cache, A_wq, A_wo,
      B_x.reshape(_B, _D), B_k_cache, B_v_cache, B_wq, B_wo)
    return out.reshape(_B, 1, 2 * _D)
```
